```python
import os as _os
_os.environ.setdefault("JAX_PLATFORMS", "cpu")
import jax
import jax.numpy as jnp

def _softmax(x, axis=-1):
    return jax.nn.softmax(x, axis=axis)
def _gelu(x):
    return jax.nn.gelu(x, approximate=True)
def _silu(x):
    return jax.nn.silu(x)
def _sigmoid(x):
    return jax.nn.sigmoid(x)
def _layernorm(x, axis=-1, eps=1e-5):
    m = jnp.mean(x, axis=axis, keepdims=True)
    v = jnp.var(x, axis=axis, keepdims=True)
    return (x - m) / jnp.sqrt(v + eps)
def _scatter_add(tgt, idx, src, axis=0):
    return tgt.at[idx].add(src)
def _segment_sum(src, seg, n):
    return jax.ops.segment_sum(src, seg, n)
class _Rng:
    def __init__(self, key):
        self._k = key
    def _next(self):
        self._k, sub = jax.random.split(self._k)
        return sub
    def normal(self, shape):
        return jax.random.normal(self._next(), shape, dtype=jnp.bfloat16)
    def randint(self, lo, hi, shape):
        return jax.random.randint(self._next(), shape, lo, hi, dtype=jnp.int32)
    def uniform(self, shape, lo=0.0, hi=1.0):
        return jax.random.uniform(self._next(), shape, jnp.bfloat16, lo, hi)
    def permutation(self, n):
        return jax.random.permutation(self._next(), n)


kernel_name = 'concat_heads__mha_block_cached__mha_block_cached__near_ridge'

def setup_inputs():
    _rng = _Rng(jax.random.key(int.from_bytes(__import__("os").urandom(4), "little")))
    _w = (lambda a: (lambda t: t.astype(jnp.bfloat16) if jnp.issubdtype(t.dtype, jnp.floating) else t)(jnp.asarray(a)))
    def _A_setup():
        B, Sq, D = 8, 160, 512
        H, Sk, Dh = 32, 512, 128
        return {
            "x": _w((lambda *s: _rng.normal(s) * 0.8)(B, Sq, D)),
            "k_cache": _w((lambda *s: _rng.normal(s) * 0.8)(B, H, Sk, Dh)),
            "v_cache": _w((lambda *s: _rng.normal(s) * 0.05)(B, H, Sk, Dh)),
            "wq": _w((lambda *s: _rng.normal(s) * 0.8)(D, H * Dh) * (D ** -0.5)),
            "wo": _w((lambda *s: _rng.normal(s) * 0.05)(H * Dh, D) * ((H * Dh) ** -0.5)),
        }
    _A_in = _A_setup()

    def _B_setup():
        B, Sq, D = 8, 160, 512
        H, Sk, Dh = 32, 512, 128
        return {
            "x": _w((lambda *s: _rng.normal(s) * 0.8)(B, Sq, D)),
            "k_cache": _w((lambda *s: _rng.normal(s) * 0.8)(B, H, Sk, Dh)),
            "v_cache": _w((lambda *s: _rng.normal(s) * 0.05)(B, H, Sk, Dh)),
            "wq": _w((lambda *s: _rng.normal(s) * 0.8)(D, H * Dh) * (D ** -0.5)),
            "wo": _w((lambda *s: _rng.normal(s) * 0.05)(H * Dh, D) * ((H * Dh) ** -0.5)),
        }
    _B_in = _B_setup()

    return {
        "A_x": _A_in["x"],
        "A_k_cache": _A_in["k_cache"],
        "A_v_cache": _A_in["v_cache"],
        "A_wq": _A_in["wq"],
        "A_wo": _A_in["wo"],
        "B_x": _B_in["x"],
        "B_k_cache": _B_in["k_cache"],
        "B_v_cache": _B_in["v_cache"],
        "B_wq": _B_in["wq"],
        "B_wo": _B_in["wo"],
    }

def reference(A_x, A_k_cache, A_v_cache, A_wq, A_wo, B_x, B_k_cache, B_v_cache, B_wq, B_wo):
    def _A_ref(x, k_cache, v_cache, wq, wo):
        B, Sq, D = x.shape
        H, Dh = 32, 128
        q = (lambda x, *d: x.transpose(*d))((x @ wq).reshape(B, Sq, H, Dh), 0, 2, 1, 3)
        scores = jnp.einsum("bhqd,bhkd->bhqk", q, k_cache) * (Dh ** -0.5)
        p = _softmax(scores, axis=-1)
        o = jnp.einsum("bhqk,bhkd->bhqd", p, v_cache)
        return (lambda x, *d: x.transpose(*d))(o, 0, 2, 1, 3).reshape(B, Sq, H * Dh) @ wo

    def _B_ref(x, k_cache, v_cache, wq, wo):
        B, Sq, D = x.shape
        H, Dh = 32, 128
        q = (lambda x, *d: x.transpose(*d))((x @ wq).reshape(B, Sq, H, Dh), 0, 2, 1, 3)
        scores = jnp.einsum("bhqd,bhkd->bhqk", q, k_cache) * (Dh ** -0.5)
        p = _softmax(scores, axis=-1)
        o = jnp.einsum("bhqk,bhkd->bhqd", p, v_cache)
        return (lambda x, *d: x.transpose(*d))(o, 0, 2, 1, 3).reshape(B, Sq, H * Dh) @ wo

    a = _A_ref(A_x, A_k_cache, A_v_cache, A_wq, A_wo)
    b = _B_ref(B_x, B_k_cache, B_v_cache, B_wq, B_wo)
    return jnp.concatenate([a, b], axis=-1)
```

```python
import os
import jax
import jax.numpy as jnp
from jax.experimental import pallas as pl
from jax.experimental.pallas import tpu as pltpu

B, SQ, D = 8, 160, 512
H, SK, DH = 32, 512, 128
M = B * SQ
LOG2E = 1.4426950408889634
QSCALE = (DH ** -0.5) * LOG2E

G = int(os.environ.get("K_G", "2"))
NS = int(os.environ.get("K_NS", "3"))
NA = int(os.environ.get("K_NA", "5"))
XC = int(os.environ.get("K_XC", "4"))
OC = int(os.environ.get("K_OC", "4"))
QPOS = int("1")
SPOS = int(os.environ.get("K_SPOS", "1"))
XBS = int(os.environ.get("K_XBS", "4"))
NOBC = int(os.environ.get("K_NOBC", "1"))
NHG = H // G
NSTEP = 2 * NHG
NW = NA + 2
NQ = NA + 1
assert NA < NHG - XBS and NS == 3


def _recip(l):
    r = pl.reciprocal(l, approx=True)
    return r * (2.0 - l * r)


def _kernel(xa, ka, va, wqa, woa, xb, kb, vb, wqb, wob, o_hbm,
            x_buf, k_buf, v_buf, wq_buf, wo_buf, q_buf, ob_buf, acc_ref, out_buf,
            sem_x, sem_k, sem_v, sem_wq, sem_wo, sem_o, sem_order):
    halves = ((xa, ka, va, wqa, woa), (xb, kb, vb, wqb, wob))

    def k_copy(half, hg, slot):
        return pltpu.make_async_copy(halves[half][1].at[:, pl.ds(hg * G, G)], k_buf.at[slot], sem_k.at[slot])

    def v_copy(half, hg, slot):
        return pltpu.make_async_copy(halves[half][2].at[:, pl.ds(hg * G, G)], v_buf.at[slot], sem_v.at[slot])

    def wq_copy(half, hg, slot):
        return pltpu.make_async_copy(halves[half][3].at[:, pl.ds(hg * (G * DH), G * DH)], wq_buf.at[slot], sem_wq.at[slot])

    def wo_copy(half, hg, slot):
        return pltpu.make_async_copy(halves[half][4].at[pl.ds(hg * (G * DH), G * DH), :], wo_buf.at[slot], sem_wo.at[slot])

    def for_step(step, fn):
        if isinstance(step, int):
            if step < NSTEP:
                fn(step // NHG, step % NHG)
            return

        @pl.when(step < NHG)
        def _():
            fn(0, step)

        @pl.when(jnp.logical_and(step >= NHG, step < NSTEP))
        def _():
            fn(1, step - NHG)

    def start_kvo(step):
        def fn(half, hg):
            k_copy(half, hg, step % NS).start()
            v_copy(half, hg, step % NS).start()
            wo_copy(half, hg, step % NS).start()
        for_step(step, fn)

    def start_wq(step):
        for_step(step, lambda half, hg: wq_copy(half, hg, step % NW).start())

    def order_barrier():
        pl.semaphore_signal(sem_order, 1)
        pl.semaphore_wait(sem_order, 1)

    XR = M // XC
    OR = M // OC
    xa_copies = [pltpu.make_async_copy(xa.at[pl.ds(c * XR, XR)], x_buf.at[0, pl.ds(c * XR, XR)], sem_x.at[c]) for c in range(XC)]
    xb_copy = pltpu.make_async_copy(xb, x_buf.at[1], sem_x.at[XC])

    def out_copy(half, c):
        return pltpu.make_async_copy(out_buf.at[half, pl.ds(c * OR, OR)],
                                     o_hbm.at[pl.ds(c * OR, OR), pl.ds(half * D, D)], sem_o.at[half, c])

    def qproj(step, r0=0, nr=M):
        q = jnp.dot(x_buf[step // NHG, pl.ds(r0, nr), :], wq_buf[step % NW],
                    preferred_element_type=jnp.float32) * QSCALE
        q_buf[step % NQ, pl.ds(r0, nr), :] = q.astype(jnp.bfloat16)

    def attention(step, hook):
        slot, qslot = step % NS, step % NQ

        def qk(b, g):
            qb = q_buf[qslot, b * SQ:(b + 1) * SQ, g * DH:(g + 1) * DH]
            return jax.lax.dot_general(qb, k_buf[slot, b, g], (((1,), (1,)), ((), ())),
                                       preferred_element_type=jnp.float32)

        def pv(b, g, s):
            m = jnp.max(s, axis=-1, keepdims=True)
            p = jnp.exp2(s - m)
            l = jnp.sum(p, axis=-1, keepdims=True)
            o = jnp.dot(p.astype(jnp.bfloat16), v_buf[slot, b, g], preferred_element_type=jnp.float32)
            o = o * _recip(l)
            ob_buf[b * SQ:(b + 1) * SQ, g * DH:(g + 1) * DH] = o.astype(jnp.bfloat16)

        units = [(b, g) for b in range(B) for g in range(G)]
        s_next = qk(*units[0])
        for i, (b, g) in enumerate(units):
            s = s_next
            if i + 1 < len(units):
                s_next = qk(*units[i + 1])
            if i == SPOS:
                hook()
            pv(b, g, s)

    def oproj(step):
        half, hg = step // NHG, step % NHG
        for c in range(OC):
            rows = pl.ds(c * OR, OR)
            contrib = jnp.dot(ob_buf[rows, :], wo_buf[step % NS], preferred_element_type=jnp.float32)
            new = jnp.where(hg == 0, 0.0, acc_ref[rows, :]) + contrib
            acc_ref[rows, :] = new
            out_buf[half, rows, :] = new.astype(jnp.bfloat16)

            @pl.when(step == NHG - 1)
            def _():
                out_copy(0, c).start()

            @pl.when(step == NSTEP - 1)
            def _():
                out_copy(1, c).start()

    def wait_kvo(step):
        k_copy(0, 0, step % NS).wait()
        v_copy(0, 0, step % NS).wait()
        wo_copy(0, 0, step % NS).wait()

    start_wq(0)
    for c in range(XC):
        xa_copies[c].start()
        order_barrier()
    for j in range(1, NA):
        start_wq(j)
    order_barrier()
    start_kvo(0)
    order_barrier()
    start_wq(NA)
    order_barrier()
    start_kvo(1)
    start_wq(NA + 1)

    wq_copy(0, 0, 0).wait()
    for c in range(XC):
        xa_copies[c].wait()
        qproj(0, c * XR, XR)

    def pro_body(j, carry):
        wq_copy(0, 0, j % NW).wait()
        qproj(j)
        return carry

    jax.lax.fori_loop(1, NA, pro_body, 0)

    def main_body(step, carry):
        def hook():
            start_wq(step + NA + 2)
            start_kvo(step + 2)

            @pl.when(step == XBS)
            def _():
                xb_copy.start()

        @pl.when(step == NHG - NA)
        def _():
            xb_copy.wait()

        wq_copy(0, 0, (step + NA) % NW).wait()
        wait_kvo(step)
        if QPOS == 0:
            qproj(step + NA)
        attention(step, hook)
        oproj(step)
        if QPOS == 1:
            qproj(step + NA)
        return carry

    jax.lax.fori_loop(0, NSTEP - NA, main_body, 0)

    def tail_body(step, carry):
        wait_kvo(step)
        attention(step, lambda: start_kvo(step + 2))
        oproj(step)
        return carry

    jax.lax.fori_loop(NSTEP - NA, NSTEP, tail_body, 0)

    for half in range(2):
        for c in range(OC):
            out_copy(half, c).wait()


@jax.jit
def pallas_concat_heads__mha_block_cached__mha_block_cached__near_ridge_kernel(
    A_x, A_k_cache, A_v_cache, A_wq, A_wo, B_x, B_k_cache, B_v_cache, B_wq, B_wo,
):
    any_spec = pl.BlockSpec(memory_space=pl.ANY)
    out = pl.pallas_call(
        _kernel,
        in_specs=[any_spec] * 10,
        out_specs=any_spec,
        out_shape=jax.ShapeDtypeStruct((M, 2 * D), jnp.bfloat16),
        scratch_shapes=[
            pltpu.VMEM((2, M, D), jnp.bfloat16),
            pltpu.VMEM((NS, B, G, SK, DH), jnp.bfloat16),
            pltpu.VMEM((NS, B, G, SK, DH), jnp.bfloat16),
            pltpu.VMEM((NW, D, G * DH), jnp.bfloat16),
            pltpu.VMEM((NS, G * DH, D), jnp.bfloat16),
            pltpu.VMEM((NQ, M, G * DH), jnp.bfloat16),
            pltpu.VMEM((M, G * DH), jnp.bfloat16),
            pltpu.VMEM((M, D), jnp.float32),
            pltpu.VMEM((2, M, D), jnp.bfloat16),
            pltpu.SemaphoreType.DMA((XC + 1,)),
            pltpu.SemaphoreType.DMA((NS,)),
            pltpu.SemaphoreType.DMA((NS,)),
            pltpu.SemaphoreType.DMA((NW,)),
            pltpu.SemaphoreType.DMA((NS,)),
            pltpu.SemaphoreType.DMA((2, OC)),
            pltpu.SemaphoreType.REGULAR,
        ],
        compiler_params=pltpu.CompilerParams(
            vmem_limit_bytes=100 * 1024 * 1024,
            disable_bounds_checks=bool(NOBC),
        ),
    )(A_x.reshape(M, D), A_k_cache, A_v_cache, A_wq, A_wo,
      B_x.reshape(M, D), B_k_cache, B_v_cache, B_wq, B_wo)
    return out.reshape(B, SQ, 2 * D)
```

```python
import jax
import jax.numpy as jnp
from jax.experimental import pallas as pl
from jax.experimental.pallas import tpu as pltpu

B, SQ, D = 8, 160, 512
H, SK, DH = 32, 512, 128
M = B * SQ
QSCALE = (DH ** -0.5) * 1.4426950408889634

G = 4
NS = 3
NA = 5
NHG = H // G
NSTEP = 2 * NHG
NW = NA + NS - 1
NQ = NA + 1
XC = 4
W0 = 2
PG = 2
OC = 8
assert (NA - 1) % PG == 0 and NA < NHG and W0 < G


def _next(slot, n):
    nxt = slot + 1
    return jnp.where(nxt == n, 0, nxt)


def _kernel(xa, ka, va, wqa, woa, xb, kb, vb, wqb, wob, o_hbm,
            x_buf, k_buf, v_buf, wq_buf, wo_buf, q_buf, ob_buf, acc_ref, out_buf,
            sem_x, sem_k, sem_v, sem_wq, sem_wo, sem_o, sem_order):
    blocks = ((xa, ka, va, wqa, woa), (xb, kb, vb, wqb, wob))

    def k_copy(blk, hg, slot):
        return pltpu.make_async_copy(blocks[blk][1].at[:, pl.ds(hg * G, G)], k_buf.at[slot], sem_k.at[slot])

    def v_copy(blk, hg, slot):
        return pltpu.make_async_copy(blocks[blk][2].at[:, pl.ds(hg * G, G)], v_buf.at[slot], sem_v.at[slot])

    def wq_copy(blk, hg, slot):
        return pltpu.make_async_copy(blocks[blk][3].at[:, pl.ds(hg * (G * DH), G * DH)], wq_buf.at[slot], sem_wq.at[slot])

    def wo_copy(blk, hg, slot):
        return pltpu.make_async_copy(blocks[blk][4].at[pl.ds(hg * (G * DH), G * DH), :], wo_buf.at[slot], sem_wo.at[slot])

    def for_step(step, fn):
        if isinstance(step, int):
            if step < NSTEP:
                fn(step // NHG, step % NHG)
            return

        @pl.when(step < NHG)
        def _():
            fn(0, step)

        @pl.when(jnp.logical_and(step >= NHG, step < NSTEP))
        def _():
            fn(1, step - NHG)

    def start_kvo(step, slot):
        def fn(blk, hg):
            k_copy(blk, hg, slot).start()
            v_copy(blk, hg, slot).start()
            wo_copy(blk, hg, slot).start()
        for_step(step, fn)

    def start_wq(step, slot):
        for_step(step, lambda blk, hg: wq_copy(blk, hg, slot).start())

    def wait_kvo(slot):
        k_copy(0, 0, slot).wait()
        v_copy(0, 0, slot).wait()
        wo_copy(0, 0, slot).wait()

    def order_barrier():
        pl.semaphore_signal(sem_order, 1)
        pl.semaphore_wait(sem_order, 1)

    xr, orows = M // XC, M // OC
    xa_copies = [pltpu.make_async_copy(xa.at[pl.ds(c * xr, xr)], x_buf.at[0, pl.ds(c * xr, xr)], sem_x.at[c])
                 for c in range(XC)]
    xb_copy = pltpu.make_async_copy(xb, x_buf.at[1], sem_x.at[XC])

    def out_copy(blk, c):
        rows = pl.ds(c * orows, orows)
        return pltpu.make_async_copy(out_buf.at[blk, rows], o_hbm.at[rows, pl.ds(blk * D, D)], sem_o)

    def qproj(blk, wslot, qslot, rows=slice(None), cols=slice(None)):
        q = jnp.dot(x_buf[blk, rows, :], wq_buf[wslot, :, cols], preferred_element_type=jnp.float32)
        q_buf[qslot, rows, cols] = (q * QSCALE).astype(jnp.bfloat16)

    def attention(slot, qslot, start_prefetch):
        def qk(b, g):
            q = q_buf[qslot, b * SQ:(b + 1) * SQ, g * DH:(g + 1) * DH]
            return jax.lax.dot_general(q, k_buf[slot, b, g], (((1,), (1,)), ((), ())),
                                       preferred_element_type=jnp.float32)

        def softmax_pv(b, g, s):
            m = jnp.max(s, axis=-1, keepdims=True)
            p = jnp.exp2(s - m)
            l = jnp.sum(p, axis=-1, keepdims=True)
            o = jnp.dot(p.astype(jnp.bfloat16), v_buf[slot, b, g], preferred_element_type=jnp.float32)
            r = pl.reciprocal(l, approx=True)
            r = r * (2.0 - l * r)
            ob_buf[b * SQ:(b + 1) * SQ, g * DH:(g + 1) * DH] = (o * r).astype(jnp.bfloat16)

        units = [(b, g) for b in range(B) for g in range(G)]
        s_next = qk(*units[0])
        for i, (b, g) in enumerate(units):
            s = s_next
            if i + 1 < len(units):
                s_next = qk(*units[i + 1])
            if i == 1:
                start_prefetch()
            softmax_pv(b, g, s)

    def oproj(step, slot):
        blk = (step >= NHG).astype(jnp.int32)
        first_of_block = jnp.logical_or(step == 0, step == NHG)
        for c in range(OC):
            rows = pl.ds(c * orows, orows)
            contrib = jnp.dot(ob_buf[rows, :], wo_buf[slot], preferred_element_type=jnp.float32)
            new = jnp.where(first_of_block, 0.0, acc_ref[rows, :]) + contrib
            acc_ref[rows, :] = new
            out_buf[blk, rows, :] = new.astype(jnp.bfloat16)

            @pl.when(step == NHG - 1)
            def _():
                out_copy(0, c).start()

            @pl.when(step == NSTEP - 1)
            def _():
                out_copy(1, c).start()

    cols0, cols1 = pl.ds(0, W0 * DH), pl.ds(W0 * DH, (G - W0) * DH)
    wq0a = pltpu.make_async_copy(wqa.at[:, cols0], wq_buf.at[0, :, cols0], sem_wq.at[0])
    wq0b = pltpu.make_async_copy(wqa.at[:, cols1], wq_buf.at[0, :, cols1], sem_wq.at[NW])
    wq0a.start()
    for c in range(XC):
        xa_copies[c].start()
        order_barrier()
    wq0b.start()
    order_barrier()
    for j in range(1, NA):
        start_wq(j, j)
        order_barrier()
    for j in range(NS - 1):
        start_kvo(j, j)
        order_barrier()
        start_wq(NA + j, NA + j)
        order_barrier()

    wq0a.wait()
    for c in range(XC):
        xa_copies[c].wait()
        qproj(0, 0, 0, pl.ds(c * xr, xr), cols0)
    wq0b.wait()
    qproj(0, 0, 0, slice(None), cols1)

    def prologue_body(i, carry):
        for u in range(PG):
            wq_copy(0, 0, 1 + i * PG + u).wait()
        for u in range(PG):
            qproj(0, 1 + i * PG + u, 1 + i * PG + u)
        return carry

    jax.lax.fori_loop(0, (NA - 1) // PG, prologue_body, 0)

    def main_body(step, carry):
        slot, slot_new, qslot, qslot_new, wslot, wslot_new = carry

        def start_prefetch():
            start_wq(step + NA + NS - 1, wslot_new)
            start_kvo(step + NS - 1, slot_new)

            @pl.when(step == 0)
            def _():
                xb_copy.start()

        @pl.when(step == NHG - NA)
        def _():
            xb_copy.wait()

        wq_copy(0, 0, wslot).wait()
        wait_kvo(slot)
        attention(slot, qslot, start_prefetch)
        oproj(step, slot)
        qproj((step >= NHG - NA).astype(jnp.int32), wslot, qslot_new)
        return _next(slot, NS), slot, _next(qslot, NQ), qslot, _next(wslot, NW), _next(wslot_new, NW)

    jax.lax.fori_loop(0, NSTEP - NA, main_body, (0, NS - 1, 0, NA, NA, (NA + NS - 1) % NW))

    def tail_body(step, carry):
        slot, slot_new, qslot = carry
        wait_kvo(slot)
        attention(slot, qslot, lambda: start_kvo(step + NS - 1, slot_new))
        oproj(step, slot)
        return _next(slot, NS), slot, _next(qslot, NQ)

    s0 = NSTEP - NA
    jax.lax.fori_loop(s0, NSTEP, tail_body, (s0 % NS, (s0 - 1) % NS, s0 % NQ))

    pltpu.make_async_copy(out_buf, out_buf, sem_o).wait()


@jax.jit
def pallas_concat_heads__mha_block_cached__mha_block_cached__near_ridge_kernel(
    A_x: jax.Array,
    A_k_cache: jax.Array,
    A_v_cache: jax.Array,
    A_wq: jax.Array,
    A_wo: jax.Array,
    B_x: jax.Array,
    B_k_cache: jax.Array,
    B_v_cache: jax.Array,
    B_wq: jax.Array,
    B_wo: jax.Array,
):
    hbm = pl.BlockSpec(memory_space=pl.ANY)
    out = pl.pallas_call(
        _kernel,
        in_specs=[hbm] * 10,
        out_specs=hbm,
        out_shape=jax.ShapeDtypeStruct((M, 2 * D), jnp.bfloat16),
        scratch_shapes=[
            pltpu.VMEM((2, M, D), jnp.bfloat16),
            pltpu.VMEM((NS, B, G, SK, DH), jnp.bfloat16),
            pltpu.VMEM((NS, B, G, SK, DH), jnp.bfloat16),
            pltpu.VMEM((NW, D, G * DH), jnp.bfloat16),
            pltpu.VMEM((NS, G * DH, D), jnp.bfloat16),
            pltpu.VMEM((NQ, M, G * DH), jnp.bfloat16),
            pltpu.VMEM((M, G * DH), jnp.bfloat16),
            pltpu.VMEM((M, D), jnp.float32),
            pltpu.VMEM((2, M, D), jnp.bfloat16),
            pltpu.SemaphoreType.DMA((XC + 1,)),
            pltpu.SemaphoreType.DMA((NS,)),
            pltpu.SemaphoreType.DMA((NS,)),
            pltpu.SemaphoreType.DMA((NW + 1,)),
            pltpu.SemaphoreType.DMA((NS,)),
            pltpu.SemaphoreType.DMA(()),
            pltpu.SemaphoreType.REGULAR,
        ],
        compiler_params=pltpu.CompilerParams(
            vmem_limit_bytes=100 * 1024 * 1024,
            disable_bounds_checks=True,
        ),
    )(A_x.reshape(M, D), A_k_cache, A_v_cache, A_wq, A_wo,
      B_x.reshape(M, D), B_k_cache, B_v_cache, B_wq, B_wo)
    return out.reshape(B, SQ, 2 * D)
```

```python
import jax
import jax.numpy as jnp
from jax.experimental import pallas as pl
from jax.experimental.pallas import tpu as pltpu

B, SQ, D = 8, 160, 512
H, SK, DH = 32, 512, 128
M = B * SQ
QSCALE = (DH ** -0.5) * 1.4426950408889634

G = 4
NS = 3
NA = 5
NHG = H // G
NSTEP = 2 * NHG
NW = NA + NS - 1
NQ = NA + 1
XC = 16
W0 = 3
WL = 2
PG = 2
OC = 8
assert (NA - 1) % PG == 0 and NA < NHG and W0 < G


def _next(slot, n):
    nxt = slot + 1
    return jnp.where(nxt == n, 0, nxt)


def _kernel(xa, ka, va, wqa, woa, xb, kb, vb, wqb, wob, o_hbm,
            x_buf, k_buf, v_buf, wq_buf, wo_buf, q_buf, ob_buf, acc_ref, out_buf,
            sem_x, sem_k, sem_v, sem_wq, sem_wo, sem_o, sem_order):
    blocks = ((xa, ka, va, wqa, woa), (xb, kb, vb, wqb, wob))

    def k_copy(blk, hg, slot):
        return pltpu.make_async_copy(blocks[blk][1].at[:, pl.ds(hg * G, G)], k_buf.at[slot], sem_k.at[slot])

    def v_copy(blk, hg, slot):
        return pltpu.make_async_copy(blocks[blk][2].at[:, pl.ds(hg * G, G)], v_buf.at[slot], sem_v.at[slot])

    def wq_copy(blk, hg, slot):
        return pltpu.make_async_copy(blocks[blk][3].at[:, pl.ds(hg * (G * DH), G * DH)], wq_buf.at[slot], sem_wq.at[slot])

    def wo_copy(blk, hg, slot):
        return pltpu.make_async_copy(blocks[blk][4].at[pl.ds(hg * (G * DH), G * DH), :], wo_buf.at[slot], sem_wo.at[slot])

    def for_step(step, fn):
        if isinstance(step, int):
            if step < NSTEP:
                fn(step // NHG, step % NHG)
            return

        @pl.when(step < NHG)
        def _():
            fn(0, step)

        @pl.when(jnp.logical_and(step >= NHG, step < NSTEP))
        def _():
            fn(1, step - NHG)

    def start_kvo(step, slot):
        def fn(blk, hg):
            k_copy(blk, hg, slot).start()
            v_copy(blk, hg, slot).start()
            wo_copy(blk, hg, slot).start()
        for_step(step, fn)

    def start_wq(step, slot):
        for_step(step, lambda blk, hg: wq_copy(blk, hg, slot).start())

    def wait_kvo(slot):
        k_copy(0, 0, slot).wait()
        v_copy(0, 0, slot).wait()
        wo_copy(0, 0, slot).wait()

    def order_barrier():
        pl.semaphore_signal(sem_order, 1)
        pl.semaphore_wait(sem_order, 1)

    xr, orows = M // XC, M // OC
    xa_copies = [pltpu.make_async_copy(xa.at[pl.ds(c * xr, xr)], x_buf.at[0, pl.ds(c * xr, xr)], sem_x.at[c])
                 for c in range(XC)]
    xb_copy = pltpu.make_async_copy(xb, x_buf.at[1], sem_x.at[XC])

    def out_copy(blk, c):
        rows = pl.ds(c * orows, orows)
        return pltpu.make_async_copy(out_buf.at[blk, rows], o_hbm.at[rows, pl.ds(blk * D, D)], sem_o)

    def qproj(blk, wslot, qslot, rows=slice(None), cols=slice(None)):
        q = jnp.dot(x_buf[blk, rows, :], wq_buf[wslot, :, cols], preferred_element_type=jnp.float32)
        q_buf[qslot, rows, cols] = (q * QSCALE).astype(jnp.bfloat16)

    def attention(slot, qslot, start_prefetch, lead=None):
        units = [(b, g) for b in range(B) for g in range(G)]

        def load_q(b, g):
            return q_buf[qslot, b * SQ:(b + 1) * SQ, g * DH:(g + 1) * DH]

        early_q = {u: load_q(*u) for u in units[:2]} if lead is not None else {}
        if lead is not None:
            lead()

        def qk(b, g):
            q = early_q[(b, g)] if (b, g) in early_q else load_q(b, g)
            return jax.lax.dot_general(q, k_buf[slot, b, g], (((1,), (1,)), ((), ())),
                                       preferred_element_type=jnp.float32)

        def softmax_pv(b, g, s):
            m = jnp.max(s, axis=-1, keepdims=True)
            p = jnp.exp2(s - m)
            l = jnp.sum(p, axis=-1, keepdims=True)
            o = jnp.dot(p.astype(jnp.bfloat16), v_buf[slot, b, g], preferred_element_type=jnp.float32)
            r = pl.reciprocal(l, approx=True)
            r = r * (2.0 - l * r)
            ob_buf[b * SQ:(b + 1) * SQ, g * DH:(g + 1) * DH] = (o * r).astype(jnp.bfloat16)

        s_next = qk(*units[0])
        for i, (b, g) in enumerate(units):
            s = s_next
            if i + 1 < len(units):
                s_next = qk(*units[i + 1])
            if i == 1:
                start_prefetch()
            softmax_pv(b, g, s)

    def oproj(step, slot):
        blk = (step >= NHG).astype(jnp.int32)
        first_of_block = jnp.logical_or(step == 0, step == NHG)
        for c in range(OC):
            rows = pl.ds(c * orows, orows)
            contrib = jnp.dot(ob_buf[rows, :], wo_buf[slot], preferred_element_type=jnp.float32)
            new = jnp.where(first_of_block, 0.0, acc_ref[rows, :]) + contrib
            acc_ref[rows, :] = new
            out_buf[blk, rows, :] = new.astype(jnp.bfloat16)

            @pl.when(step == NHG - 1)
            def _():
                out_copy(0, c).start()

            @pl.when(step == NSTEP - 1)
            def _():
                out_copy(1, c).start()

    cols0, cols1 = pl.ds(0, W0 * DH), pl.ds(W0 * DH, (G - W0) * DH)
    wq0a = pltpu.make_async_copy(wqa.at[:, cols0], wq_buf.at[0, :, cols0], sem_wq.at[0])
    wq0b = pltpu.make_async_copy(wqa.at[:, cols1], wq_buf.at[0, :, cols1], sem_wq.at[NW])
    wq0a.start()
    for c in range(XC):
        xa_copies[c].start()
        order_barrier()
    wq0b.start()
    order_barrier()
    for j in range(1, NA):
        start_wq(j, j)
        order_barrier()
    for j in range(NS - 1):
        start_kvo(j, j)
        order_barrier()
        start_wq(NA + j, NA + j)
        order_barrier()

    wq0a.wait()
    for c in range(XC):
        xa_copies[c].wait()
        qproj(0, 0, 0, pl.ds(c * xr, xr), cols0)
    wq0b.wait()
    qproj(0, 0, 0, slice(None), cols1)

    def prologue_body(i, carry):
        for u in range(PG):
            wq_copy(0, 0, 1 + i * PG + u).wait()
        for u in range(PG):
            qproj(0, 1 + i * PG + u, 1 + i * PG + u)
        return carry

    jax.lax.fori_loop(0, (NA - 1) // PG, prologue_body, 0)

    def main_body(step, carry):
        slot, slot_new, qslot, qslot_new, wslot, wslot_new = carry

        def start_prefetch():
            start_wq(step + NA + NS - 1, wslot_new)
            start_kvo(step + NS - 1, slot_new)

            @pl.when(step == 0)
            def _():
                xb_copy.start()

        @pl.when(step == NHG - NA)
        def _():
            xb_copy.wait()

        wq_copy(0, 0, wslot).wait()
        wait_kvo(slot)
        qblk = (step >= NHG - NA).astype(jnp.int32)
        attention(slot, qslot, start_prefetch,
                  lead=lambda: qproj(qblk, wslot, qslot_new, cols=pl.ds(0, WL * DH)))
        qproj(qblk, wslot, qslot_new, cols=pl.ds(WL * DH, (G - WL) * DH))
        oproj(step, slot)
        return _next(slot, NS), slot, _next(qslot, NQ), qslot, _next(wslot, NW), _next(wslot_new, NW)

    jax.lax.fori_loop(0, NSTEP - NA, main_body, (0, NS - 1, 0, NA, NA, (NA + NS - 1) % NW))

    def tail_body(step, carry):
        slot, slot_new, qslot = carry
        wait_kvo(slot)
        attention(slot, qslot, lambda: start_kvo(step + NS - 1, slot_new))
        oproj(step, slot)
        return _next(slot, NS), slot, _next(qslot, NQ)

    s0 = NSTEP - NA
    jax.lax.fori_loop(s0, NSTEP, tail_body, (s0 % NS, (s0 - 1) % NS, s0 % NQ))

    pltpu.make_async_copy(out_buf, out_buf, sem_o).wait()


@jax.jit
def pallas_concat_heads__mha_block_cached__mha_block_cached__near_ridge_kernel(
    A_x: jax.Array,
    A_k_cache: jax.Array,
    A_v_cache: jax.Array,
    A_wq: jax.Array,
    A_wo: jax.Array,
    B_x: jax.Array,
    B_k_cache: jax.Array,
    B_v_cache: jax.Array,
    B_wq: jax.Array,
    B_wo: jax.Array,
):
    hbm = pl.BlockSpec(memory_space=pl.ANY)
    out = pl.pallas_call(
        _kernel,
        in_specs=[hbm] * 10,
        out_specs=hbm,
        out_shape=jax.ShapeDtypeStruct((M, 2 * D), jnp.bfloat16),
        scratch_shapes=[
            pltpu.VMEM((2, M, D), jnp.bfloat16),
            pltpu.VMEM((NS, B, G, SK, DH), jnp.bfloat16),
            pltpu.VMEM((NS, B, G, SK, DH), jnp.bfloat16),
            pltpu.VMEM((NW, D, G * DH), jnp.bfloat16),
            pltpu.VMEM((NS, G * DH, D), jnp.bfloat16),
            pltpu.VMEM((NQ, M, G * DH), jnp.bfloat16),
            pltpu.VMEM((M, G * DH), jnp.bfloat16),
            pltpu.VMEM((M, D), jnp.float32),
            pltpu.VMEM((2, M, D), jnp.bfloat16),
            pltpu.SemaphoreType.DMA((XC + 1,)),
            pltpu.SemaphoreType.DMA((NS,)),
            pltpu.SemaphoreType.DMA((NS,)),
            pltpu.SemaphoreType.DMA((NW + 1,)),
            pltpu.SemaphoreType.DMA((NS,)),
            pltpu.SemaphoreType.DMA(()),
            pltpu.SemaphoreType.REGULAR,
        ],
        compiler_params=pltpu.CompilerParams(
            vmem_limit_bytes=100 * 1024 * 1024,
            disable_bounds_checks=True,
            flags={"XLA_TPU_RESCHEDULE_DMA_DONES": True},
        ),
    )(A_x.reshape(M, D), A_k_cache, A_v_cache, A_wq, A_wo,
      B_x.reshape(M, D), B_k_cache, B_v_cache, B_wq, B_wo)
    return out.reshape(B, SQ, 2 * D)
```

```python
import jax
import jax.numpy as jnp
from jax.experimental import pallas as pl
from jax.experimental.pallas import tpu as pltpu

B, SQ, D = 8, 160, 512
H, SK, DH = 32, 512, 128
M = B * SQ
QSCALE = (DH ** -0.5) * 1.4426950408889634

G = 4
NS = 3
NA = 5
NHG = H // G
NSTEP = 2 * NHG
NW = NA + NS
NQ = NA + 1
WL = 2
XC = 16
W0 = 3
PG = 2
OC = 8
assert (NA - 1) % PG == 0 and NA < NHG <= NSTEP - NA and W0 < G and WL < G


def _next(slot, n):
    nxt = slot + 1
    return jnp.where(nxt == n, 0, nxt)


def _kernel(xa, ka, va, wqa, woa, xb, kb, vb, wqb, wob, o_hbm,
            x_buf, k_buf, v_buf, wq_buf, wo_buf, q_buf, ob_buf, acc_ref, out_buf,
            sem_x, sem_k, sem_v, sem_wq, sem_wo, sem_o, sem_order):
    blocks = ((xa, ka, va, wqa, woa), (xb, kb, vb, wqb, wob))

    def k_copy(blk, hg, slot):
        return pltpu.make_async_copy(blocks[blk][1].at[:, pl.ds(hg * G, G)], k_buf.at[slot], sem_k.at[slot])

    def v_copy(blk, hg, slot):
        return pltpu.make_async_copy(blocks[blk][2].at[:, pl.ds(hg * G, G)], v_buf.at[slot], sem_v.at[slot])

    def wq_copy(blk, hg, slot):
        return pltpu.make_async_copy(blocks[blk][3].at[:, pl.ds(hg * (G * DH), G * DH)], wq_buf.at[slot], sem_wq.at[slot])

    def wo_copy(blk, hg, slot):
        return pltpu.make_async_copy(blocks[blk][4].at[pl.ds(hg * (G * DH), G * DH), :], wo_buf.at[slot], sem_wo.at[slot])

    def for_step(step, fn):
        if isinstance(step, int):
            if step < NSTEP:
                fn(step // NHG, step % NHG)
            return

        @pl.when(step < NHG)
        def _():
            fn(0, step)

        @pl.when(jnp.logical_and(step >= NHG, step < NSTEP))
        def _():
            fn(1, step - NHG)

    def start_kvo(step, slot):
        def fn(blk, hg):
            k_copy(blk, hg, slot).start()
            v_copy(blk, hg, slot).start()
            wo_copy(blk, hg, slot).start()
        for_step(step, fn)

    def start_wq(step, slot):
        for_step(step, lambda blk, hg: wq_copy(blk, hg, slot).start())

    def wait_kvo(slot):
        k_copy(0, 0, slot).wait()
        v_copy(0, 0, slot).wait()
        wo_copy(0, 0, slot).wait()

    def order_barrier():
        pl.semaphore_signal(sem_order, 1)
        pl.semaphore_wait(sem_order, 1)

    xr, orows = M // XC, M // OC
    xa_copies = [pltpu.make_async_copy(xa.at[pl.ds(c * xr, xr)], x_buf.at[0, pl.ds(c * xr, xr)], sem_x.at[c])
                 for c in range(XC)]
    xb_copy = pltpu.make_async_copy(xb, x_buf.at[1], sem_x.at[XC])
    outa_copy = pltpu.make_async_copy(out_buf.at[0], o_hbm.at[:, pl.ds(0, D)], sem_o)

    def outb_copy(c):
        rows = pl.ds(c * orows, orows)
        return pltpu.make_async_copy(out_buf.at[1, rows], o_hbm.at[rows, pl.ds(D, D)], sem_o)

    def qproj(blk, wslot, qslot, rows=slice(None), cols=slice(None)):
        q = jnp.dot(x_buf[blk, rows, :], wq_buf[wslot, :, cols], preferred_element_type=jnp.float32)
        q_buf[qslot, rows, cols] = (q * QSCALE).astype(jnp.bfloat16)

    def attention(slot, qslot, lead=None):
        units = [(b, g) for g in range(G) for b in range(B)]

        def load_q(b, g):
            return q_buf[qslot, b * SQ:(b + 1) * SQ, g * DH:(g + 1) * DH]

        early_q = {u: load_q(*u) for u in units[:2]} if lead is not None else {}
        if lead is not None:
            lead()

        def qk(b, g):
            q = early_q[(b, g)] if (b, g) in early_q else load_q(b, g)
            return jax.lax.dot_general(q, k_buf[slot, b, g], (((1,), (1,)), ((), ())),
                                       preferred_element_type=jnp.float32)

        def softmax_pv(b, g, s):
            m = jnp.max(s, axis=-1, keepdims=True)
            p = jnp.exp2(s - m)
            l = jnp.sum(p, axis=-1, keepdims=True)
            o = jnp.dot(p.astype(jnp.bfloat16), v_buf[slot, b, g], preferred_element_type=jnp.float32)
            r = pl.reciprocal(l, approx=True)
            r = r * (2.0 - l * r)
            ob_buf[b * SQ:(b + 1) * SQ, g * DH:(g + 1) * DH] = (o * r).astype(jnp.bfloat16)

        s_next = qk(*units[0])
        for i, (b, g) in enumerate(units):
            s = s_next
            if i + 1 < len(units):
                s_next = qk(*units[i + 1])
            softmax_pv(b, g, s)

    def oproj(step, slot, write_chunks):
        blk = (step >= NHG).astype(jnp.int32)
        first_of_block = jnp.logical_or(step == 0, step == NHG)
        for c in range(OC):
            rows = pl.ds(c * orows, orows)
            contrib = jnp.dot(ob_buf[rows, :], wo_buf[slot], preferred_element_type=jnp.float32)
            new = jnp.where(first_of_block, 0.0, acc_ref[rows, :]) + contrib
            acc_ref[rows, :] = new
            out_buf[blk, rows, :] = new.astype(jnp.bfloat16)
            if write_chunks:
                @pl.when(step == NSTEP - 1)
                def _():
                    outb_copy(c).start()

    cols0, cols1 = pl.ds(0, W0 * DH), pl.ds(W0 * DH, (G - W0) * DH)
    wq0a = pltpu.make_async_copy(wqa.at[:, cols0], wq_buf.at[0, :, cols0], sem_wq.at[0])
    wq0b = pltpu.make_async_copy(wqa.at[:, cols1], wq_buf.at[0, :, cols1], sem_wq.at[NW])
    wq0a.start()
    for c in range(XC):
        xa_copies[c].start()
        order_barrier()
    wq0b.start()
    order_barrier()
    for j in range(1, NA):
        start_wq(j, j)
        order_barrier()
    for j in range(NS):
        start_kvo(j, j)
        order_barrier()
        start_wq(NA + j, NA + j)
        order_barrier()

    wq0a.wait()
    for c in range(XC):
        xa_copies[c].wait()
        qproj(0, 0, 0, pl.ds(c * xr, xr), cols0)
    wq0b.wait()
    qproj(0, 0, 0, cols=cols1)

    def prologue_body(i, carry):
        for u in range(PG):
            wq_copy(0, 0, 1 + i * PG + u).wait()
        for u in range(PG):
            qproj(0, 1 + i * PG + u, 1 + i * PG + u)
        return carry

    jax.lax.fori_loop(0, (NA - 1) // PG, prologue_body, 0)

    def main_body(step, carry):
        slot, qslot, qslot_new, wslot, wslot_old = carry

        @pl.when(step == NHG - NA)
        def _():
            xb_copy.wait()

        wq_copy(0, 0, wslot).wait()
        wait_kvo(slot)
        qblk = (step >= NHG - NA).astype(jnp.int32)
        attention(slot, qslot, lead=lambda: qproj(qblk, wslot, qslot_new, cols=pl.ds(0, WL * DH)))
        qproj(qblk, wslot, qslot_new, cols=pl.ds(WL * DH, (G - WL) * DH))
        oproj(step, slot, write_chunks=False)

        @pl.when(step == NHG - 1)
        def _():
            outa_copy.start()

        start_kvo(step + NS, slot)
        start_wq(step + NA + NS, wslot_old)

        @pl.when(step == 0)
        def _():
            xb_copy.start()

        return _next(slot, NS), _next(qslot, NQ), qslot, _next(wslot, NW), _next(wslot_old, NW)

    jax.lax.fori_loop(0, NSTEP - NA, main_body, (0, 0, NA, NA, 0))

    def tail_body(step, carry):
        slot, qslot = carry
        wait_kvo(slot)
        attention(slot, qslot)
        oproj(step, slot, write_chunks=True)
        start_kvo(step + NS, slot)
        return _next(slot, NS), _next(qslot, NQ)

    s0 = NSTEP - NA
    jax.lax.fori_loop(s0, NSTEP, tail_body, (s0 % NS, s0 % NQ))

    pltpu.make_async_copy(out_buf, out_buf, sem_o).wait()


@jax.jit
def pallas_concat_heads__mha_block_cached__mha_block_cached__near_ridge_kernel(
    A_x: jax.Array,
    A_k_cache: jax.Array,
    A_v_cache: jax.Array,
    A_wq: jax.Array,
    A_wo: jax.Array,
    B_x: jax.Array,
    B_k_cache: jax.Array,
    B_v_cache: jax.Array,
    B_wq: jax.Array,
    B_wo: jax.Array,
):
    hbm = pl.BlockSpec(memory_space=pl.ANY)
    out = pl.pallas_call(
        _kernel,
        in_specs=[hbm] * 10,
        out_specs=hbm,
        out_shape=jax.ShapeDtypeStruct((M, 2 * D), jnp.bfloat16),
        scratch_shapes=[
            pltpu.VMEM((2, M, D), jnp.bfloat16),
            pltpu.VMEM((NS, B, G, SK, DH), jnp.bfloat16),
            pltpu.VMEM((NS, B, G, SK, DH), jnp.bfloat16),
            pltpu.VMEM((NW, D, G * DH), jnp.bfloat16),
            pltpu.VMEM((NS, G * DH, D), jnp.bfloat16),
            pltpu.VMEM((NQ, M, G * DH), jnp.bfloat16),
            pltpu.VMEM((M, G * DH), jnp.bfloat16),
            pltpu.VMEM((M, D), jnp.float32),
            pltpu.VMEM((2, M, D), jnp.bfloat16),
            pltpu.SemaphoreType.DMA((XC + 1,)),
            pltpu.SemaphoreType.DMA((NS,)),
            pltpu.SemaphoreType.DMA((NS,)),
            pltpu.SemaphoreType.DMA((NW + 1,)),
            pltpu.SemaphoreType.DMA((NS,)),
            pltpu.SemaphoreType.DMA(()),
            pltpu.SemaphoreType.REGULAR,
        ],
        compiler_params=pltpu.CompilerParams(
            vmem_limit_bytes=100 * 1024 * 1024,
            disable_bounds_checks=True,
            disable_semaphore_checks=True,
            flags={"XLA_TPU_RESCHEDULE_DMA_DONES": True},
        ),
    )(A_x.reshape(M, D), A_k_cache, A_v_cache, A_wq, A_wo,
      B_x.reshape(M, D), B_k_cache, B_v_cache, B_wq, B_wo)
    return out.reshape(B, SQ, 2 * D)
```
